```python
import jax
import jax.numpy as jnp

def _softmax(x, axis=-1):
    return jax.nn.softmax(x, axis=axis)
def _gelu(x):
    return jax.nn.gelu(x, approximate=True)
def _silu(x):
    return jax.nn.silu(x)
def _sigmoid(x):
    return jax.nn.sigmoid(x)
def _layernorm(x, axis=-1, eps=1e-5):
    m = jnp.mean(x, axis=axis, keepdims=True)
    v = jnp.var(x, axis=axis, keepdims=True)
    return (x - m) / jnp.sqrt(v + eps)
def _scatter_add(tgt, idx, src, axis=0):
    return tgt.at[idx].add(src)
def _segment_sum(src, seg, n):
    return jax.ops.segment_sum(src, seg, n)
class _Rng:
    def __init__(self, key):
        self._k = key
    def _next(self):
        self._k, sub = jax.random.split(self._k)
        return sub
    def normal(self, shape):
        return jax.random.normal(self._next(), shape, dtype=jnp.bfloat16)
    def randint(self, lo, hi, shape):
        return jax.random.randint(self._next(), shape, lo, hi, dtype=jnp.int32)
    def uniform(self, shape, lo=0.0, hi=1.0):
        return jax.random.uniform(self._next(), shape, jnp.bfloat16, lo, hi)
    def permutation(self, n):
        return jax.random.permutation(self._next(), n)


kernel_name = 'recurrent_scan__linear_kernel_hedgehog__dense_activation_relu__prompt'

def _fwd_setup_inputs():
    _rng = _Rng(jax.random.key(int.from_bytes(__import__("os").urandom(4), "little")))
    _w = (lambda a: (lambda t: t.astype(jnp.bfloat16) if jnp.issubdtype(t.dtype, jnp.floating) else t)(jnp.asarray(a)))
    def _A_setup():
        B, S, D, H = 1, 2048, 1024, 32
        Dh = D // H
        return {
            "x": _w((lambda *s: _rng.normal(s) * 0.05)(B, S, D)),
            "wqkv": _w((lambda *s: _rng.normal(s) * 0.05)(D, 3 * D)),
            "w_phi": _w((lambda *s: _rng.normal(s) * 0.05)(H, Dh, Dh) * (Dh ** -0.5)),
            "wo": _w((lambda *s: _rng.normal(s) * 0.05)(D, D)),
        }
    _A_in = _A_setup()

    def _B_setup():
        B, S, D, Dff = 1, 2048, 1024, 3584
        return {
            "x": _w((lambda *s: _rng.normal(s) * 0.05)(B, S, D)),
            "w1": _w((lambda *s: _rng.normal(s) * 0.05)(D, Dff)),
            "w2": _w((lambda *s: _rng.normal(s) * 0.05)(Dff, D)),
        }
    _B_in = _B_setup()

    return {
        "A_x": _A_in["x"],
        "A_wqkv": _A_in["wqkv"],
        "A_w_phi": _A_in["w_phi"],
        "A_wo": _A_in["wo"],
        "B_x": _B_in["x"],
        "B_w1": _B_in["w1"],
        "B_w2": _B_in["w2"],
    }

def _fwd_reference(A_x, A_wqkv, A_w_phi, A_wo, B_x, B_w1, B_w2):
    def _A_ref(x, wqkv, w_phi, wo):
        B, S, D = x.shape
        H = 32; Dh = D // H
        qkv = (lambda x, *d: x.transpose(*d))((x @ wqkv).reshape(B, S, 3, H, Dh), 2, 0, 3, 1, 4)
        q, k, v = qkv[0], qkv[1], qkv[2]
        pq = jnp.einsum("bhsd,hdf->bhsf", q, w_phi)
        pk = jnp.einsum("bhsd,hdf->bhsf", k, w_phi)
        phi_q = jnp.concatenate([_softmax(pq, axis=-1), _softmax(-pq, axis=-1)], axis=-1)
        phi_k = jnp.concatenate([_softmax(pk, axis=-1), _softmax(-pk, axis=-1)], axis=-1)
        kv = jnp.einsum("bhsf,bhsd->bhfd", phi_k, v)
        z  = jnp.einsum("bhsf->bhf", phi_k)
        num = jnp.einsum("bhqf,bhfd->bhqd", phi_q, kv)
        den = jnp.einsum("bhqf,bhf->bhq", phi_q, z)[..., None] + 1e-6
        o = num / den
        return (lambda x, *d: x.transpose(*d))(o, 0, 2, 1, 3).reshape(B, S, D) @ wo

    def _B_ref(x, w1, w2):
        h = jnp.einsum("bsd,df->bsf", x, w1)
        zero = jnp.zeros_like(h)
        h = jnp.maximum(h, zero)
        return jnp.einsum("bsf,fd->bsd", h, w2)

    x = A_x
    xn = _layernorm(x, axis=-1)
    s = _A_ref(xn, A_wqkv, A_w_phi, A_wo)
    g = _silu(_B_ref(xn, B_w1, B_w2))
    return x + s * g


def setup_inputs():
    _inp = _fwd_setup_inputs()
    _gk = jax.random.fold_in(jax.random.key(int.from_bytes(__import__("os").urandom(4), "little")), 2**31 - 1)
    _shapes = [[1, 2048, 1024]]
    _dtypes = ['bfloat16']
    _gks = jax.random.split(_gk, len(_shapes))
    _gs = [jax.random.normal(k, s, dtype=jnp.dtype(d)) * 0.05 for k, s, d in zip(_gks, _shapes, _dtypes)]
    _inp["grad_out"] = _gs[0]
    return _inp

def reference(A_x, A_wqkv, A_w_phi, A_wo, B_w1, B_w2, B_x, grad_out):
    _const = dict(B_x=B_x)
    def _f(*_d):
        return _fwd_reference(**{'A_x': _d[0], 'A_wqkv': _d[1], 'A_w_phi': _d[2], 'A_wo': _d[3], 'B_w1': _d[4], 'B_w2': _d[5], **_const})
    _out, _vjp = jax.vjp(_f, A_x, A_wqkv, A_w_phi, A_wo, B_w1, B_w2)
    _grads = _vjp(grad_out)
    _out0 = jnp.asarray(_out)
    return (_out0, *[jnp.asarray(_g) for _g in _grads])
```

```python
import jax
import jax.numpy as jnp
from jax import lax
import jax.experimental.pallas as pl
import jax.experimental.pallas.tpu as pltpu

S, D, H, DH, F = 2048, 1024, 32, 32, 3584
T = 512
NT_ = S // T
FC = 512
NC = F // FC
G = D // 128
TM = 512
BF, F32 = jnp.bfloat16, jnp.float32


def _nn(a, b):
    return lax.dot_general(a, b, (((1,), (0,)), ((), ())), preferred_element_type=F32)


def _nt(a, b):
    return lax.dot_general(a, b, (((1,), (1,)), ((), ())), preferred_element_type=F32)


def _tn(a, b):
    return lax.dot_general(a, b, (((0,), (0,)), ((), ())), preferred_element_type=F32)


def _rows(i, n):
    return pl.ds(pl.multiple_of(i * n, n), n)


def _seg(op, p4):
    return op(op(p4, axis=1), axis=1, keepdims=True)


def _dual_softmax(p):
    p4 = p.reshape(4, 4, 8, p.shape[-1])
    ep = jnp.exp(p4 - _seg(jnp.max, p4)[:, None])
    en = jnp.exp(_seg(jnp.min, p4)[:, None] - p4)
    return ep * (1.0 / _seg(jnp.sum, ep))[:, None], en * (1.0 / _seg(jnp.sum, en))[:, None]


def _dual_softmax_bwd(fp, fn, dp, dn):
    tp, tn = fp * dp, fn * dn
    r = (tp - fp * _seg(jnp.sum, tp)[:, None]) - (tn - fn * _seg(jnp.sum, tn)[:, None])
    return r.reshape(128, r.shape[-1])


def _fold_lanes(v):
    out = v[..., 0:128]
    for i in range(1, v.shape[-1] // 128):
        out = out + v[..., i * 128:(i + 1) * 128]
    return out


def _lane_total(v):
    return jnp.broadcast_to(jnp.sum(v, axis=-1, keepdims=True), v.shape)


def _tile4(z, t):
    return jnp.concatenate([z] * (t // 128), axis=-1).reshape(4, 4, 8, t)


def _diag_mask(rows):
    r = lax.broadcasted_iota(jnp.int32, (rows, 128), 0)
    c = lax.broadcasted_iota(jnp.int32, (rows, 128), 1)
    return ((r % 128) // DH) == (c // DH)


def _kernel(x_hbm, wqkv_hbm, wphi_ref, wo_hbm, w1_hbm, w2_hbm, go_hbm,
            out_hbm, dx_hbm, dwqkv_hbm, dwphi_ref, dwo_hbm, dw1_hbm, dw2_hbm,
            xb, gob, xn, xnT, rstd, wqkv, wall, wt, bd, wo, w1, w2, big, acc,
            phik, phiq, vT, oT, dy, dnT, dh, kvb, zb, rden,
            s_x, s_go, s_qkv, s_wo, s_w1, s_w2):
    x_cp = lambda t: pltpu.make_async_copy(x_hbm.at[_rows(t, T)], xb.at[_rows(t, T)], s_x.at[t])
    out_cp = lambda t: pltpu.make_async_copy(xb.at[_rows(t, T)], out_hbm.at[_rows(t, T)], s_x.at[t])
    go_cp = lambda t: pltpu.make_async_copy(go_hbm.at[_rows(t, T)], gob.at[_rows(t, T)], s_go.at[t])
    dx_cp = lambda t: pltpu.make_async_copy(gob.at[_rows(t, T)], dx_hbm.at[_rows(t, T)], s_go.at[t])
    cols = lambda j, g: pl.ds(pl.multiple_of(j * D + g * 128, 128), 128)
    qkv_cp = lambda j, g: pltpu.make_async_copy(wqkv_hbm.at[:, cols(j, g)], wqkv.at[j, g], s_qkv.at[j * G + g])
    dqkv_cp = lambda j, g: pltpu.make_async_copy(wqkv.at[j, g], dwqkv_hbm.at[:, cols(j, g)], s_qkv.at[j * G + g])
    wo_cp = pltpu.make_async_copy(wo_hbm, wo, s_wo.at[0])
    dwo_cp = pltpu.make_async_copy(wo, dwo_hbm, s_wo.at[0])
    w1_cp = lambda c: pltpu.make_async_copy(w1_hbm.at[:, _rows(c, FC)], w1.at[c], s_w1.at[c])
    dw1_cp = lambda c: pltpu.make_async_copy(w1.at[c], dw1_hbm.at[:, _rows(c, FC)], s_w1.at[c])
    w2_cp = lambda c: pltpu.make_async_copy(w2_hbm.at[_rows(c, FC)], w2.at[c], s_w2.at[c])
    dw2_cp = lambda c: pltpu.make_async_copy(w2.at[c], dw2_hbm.at[_rows(c, FC)], s_w2.at[c])
    I = jnp.int32

    for t in range(NT_):
        x_cp(I(t)).start()
    w1_cp(I(0)).start()
    w2_cp(I(0)).start()

    def ln(t, _):
        x_cp(t).wait()
        r = _rows(t, T)
        xv = xb[r, :].astype(F32)
        xc = xv - jnp.mean(xv, axis=-1, keepdims=True)
        rs = 1.0 / jnp.sqrt(jnp.mean(xc * xc, axis=-1, keepdims=True) + 1e-5)
        n = xc * rs
        rstd[r, :] = rs
        xn[r, :] = n.astype(BF)
        xnT[:, r] = n.T.astype(BF)
        acc[r, :] = jnp.zeros((T, D), F32)

    lax.fori_loop(0, NT_, ln, None)
    for c in range(1, NC):
        w1_cp(I(c)).start()
        w2_cp(I(c)).start()
    for j in range(3):
        for g in range(G):
            qkv_cp(j, I(g)).start()
    wo_cp.start()
    for t in range(NT_):
        go_cp(I(t)).start()

    def ffn_fwd(c, _):
        w1_cp(c).wait()
        w2_cp(c).wait()
        for m in range(S // TM):
            r = pl.ds(m * TM, TM)
            h = _nn(xn[r, :], w1[c])
            bits = jnp.where(h < 0, I(-2 ** 31), pltpu.bitcast(h, I) & I(2 ** 31 - 1))
            a = pltpu.bitcast(bits, F32).astype(BF)
            big[_rows(c * (S // TM) + m, TM), :] = a
            acc[r, :] += _nn(a, w2[c])

    lax.fori_loop(0, NC, ffn_fwd, None)

    for j in range(3):
        for g in range(G):
            qkv_cp(j, I(g)).wait()
    for g in range(G):
        wp = wphi_ref[pl.ds(g * 128, 128), :].astype(F32)
        b = jnp.where(_diag_mask(128), jnp.concatenate([wp] * 4, axis=1), 0.0).astype(BF)
        bd[g] = b
        for j in range(3):
            w = _nn(wqkv[j, g], b) if j < 2 else wqkv[j, g].astype(F32)
            wall[:, pl.ds(g * 384 + j * 128, 128)] = w.astype(BF)
            wt[pl.ds(g * 384 + j * 128, 128), :] = w.T.astype(BF)

    def att_fwd(g, _):
        kv = jnp.zeros((256, 128), F32)
        zp = jnp.zeros((128, 128), F32)
        zn = jnp.zeros((128, 128), F32)
        for t in range(NT_):
            r = _nn(wt[_rows(g, 384), :], xnT[:, pl.ds(t * T, T)])
            qp, qn = _dual_softmax(r[0:128])
            phiq[t, g, 0:128, :] = qp.reshape(128, T).astype(BF)
            phiq[t, g, 128:256, :] = qn.reshape(128, T).astype(BF)
            kp, kn = _dual_softmax(r[128:256])
            kp, kn = kp.reshape(128, T), kn.reshape(128, T)
            zp, zn = zp + _fold_lanes(kp), zn + _fold_lanes(kn)
            pk = jnp.concatenate([kp.astype(BF), kn.astype(BF)], axis=0)
            phik[t, g] = pk
            v = r[256:384].astype(BF)
            vT[t, g] = v
            kv = kv + _nt(pk, v)
        kv = jnp.where(_diag_mask(256), kv, 0.0)
        zp, zn = _lane_total(zp), _lane_total(zn)
        kvb[g] = kv.astype(BF)
        zb[g, 0:128, :] = zp
        zb[g, 128:256, :] = zn
        kvt = kv.T.astype(BF)
        zp4, zn4 = _tile4(zp, T), _tile4(zn, T)
        for t in range(NT_):
            pq = phiq[t, g]
            num = _nn(kvt, pq).reshape(4, 4, 8, T)
            pf = pq.astype(F32)
            den = _seg(jnp.sum, pf[0:128].reshape(4, 4, 8, T) * zp4 + pf[128:256].reshape(4, 4, 8, T) * zn4) + 1e-6
            rd = 1.0 / den
            rden[t, _rows(g, 4)] = jnp.broadcast_to(rd, (4, 8, T))
            oT[t, _rows(g, 128), :] = (num * rd[:, None]).reshape(128, T).astype(BF)

    lax.fori_loop(0, G, att_fwd, None)

    wo_cp.wait()
    ds = wt

    def gate(t, _):
        go_cp(t).wait()
        r = _rows(t, T)
        o = oT[t]
        s = _tn(o, wo[...])
        y = acc[r, :]
        gv = gob[r, :].astype(F32)
        sig = jax.nn.sigmoid(y)
        gt = y * sig
        xb[r, :] = (xb[r, :].astype(F32) + s * gt).astype(BF)
        out_cp(t).start()
        dsv = (gv * gt).astype(BF)
        ds[r, :] = dsv
        dy[r, :] = (gv * s * (sig + gt * (1.0 - sig))).astype(BF)
        acc[r, :] = jnp.zeros((T, D), F32)
        rd = rden[t]
        dn = _nt(wo[...], dsv).reshape(H, 4, 8, T) * rd[:, None]
        dnT[t] = dn.reshape(D, T).astype(BF)
        dd = -_seg(jnp.sum, dn * o.astype(F32).reshape(H, 4, 8, T))
        rden[t] = jnp.broadcast_to(dd, (H, 8, T))

    lax.fori_loop(0, NT_, gate, None)

    dwo = _nn(oT[0], ds[pl.ds(0, T), :])
    for t in range(1, NT_):
        dwo = dwo + _nn(oT[t], ds[pl.ds(t * T, T), :])
    wo[...] = dwo.astype(BF)
    dwo_cp.start()

    def ffn_bwd(c, _):
        for m in range(S // TM):
            r = pl.ds(m * TM, TM)
            da = _nt(dy[r, :], w2[c])
            bits = pltpu.bitcast(big[_rows(c * (S // TM) + m, TM), :].astype(F32), I)
            d = jnp.where(bits < 0, 0.0, jnp.where(bits == 0, 0.5 * da, da)).astype(BF)
            dh[r, :] = d
            acc[r, :] += _nt(d, w1[c])
        w1[c] = _nn(xnT[...], dh[...]).astype(BF)
        dw1_cp(c).start()
        w2[c] = _tn(big[_rows(c, S), :], dy[...]).astype(BF)
        dw2_cp(c).start()

    lax.fori_loop(0, NC, ffn_bwd, None)

    def att_bwd(g, _):
        kvv = kvb[g]
        zp4, zn4 = _tile4(zb[g, 0:128, :], T), _tile4(zb[g, 128:256, :], T)
        dkv = jnp.zeros((256, 128), F32)
        dzp = jnp.zeros((128, 128), F32)
        dzn = jnp.zeros((128, 128), F32)
        prow = lambda t, j: _rows(t * (3 * G) + g * 3 + j, 128)
        for t in range(NT_):
            dn = dnT[t, _rows(g, 128), :]
            dd = rden[t, _rows(g, 4)][:, None]
            pq = phiq[t, g]
            dphi = _nn(kvv, dn)
            dkv = dkv + _nt(pq, dn)
            pf = pq.astype(F32)
            fp, fn = pf[0:128].reshape(4, 4, 8, T), pf[128:256].reshape(4, 4, 8, T)
            dzp = dzp + _fold_lanes((fp * dd).reshape(128, T))
            dzn = dzn + _fold_lanes((fn * dd).reshape(128, T))
            dp = dphi[0:128].reshape(4, 4, 8, T) + zp4 * dd
            dm = dphi[128:256].reshape(4, 4, 8, T) + zn4 * dd
            big[prow(t, 0), :] = _dual_softmax_bwd(fp, fn, dp, dm).astype(BF)
        dkv = jnp.where(_diag_mask(256), dkv, 0.0)
        dkvb, dkvt = dkv.astype(BF), dkv.T.astype(BF)
        dzp4, dzn4 = _tile4(_lane_total(dzp), T), _tile4(_lane_total(dzn), T)
        dw = jnp.zeros((D, 384), F32)
        for t in range(NT_):
            pk = phik[t, g]
            dphi = _nn(dkvb, vT[t, g])
            big[prow(t, 2), :] = _nn(dkvt, pk).astype(BF)
            pf = pk.astype(F32)
            fp, fn = pf[0:128].reshape(4, 4, 8, T), pf[128:256].reshape(4, 4, 8, T)
            dp = dphi[0:128].reshape(4, 4, 8, T) + dzp4
            dm = dphi[128:256].reshape(4, 4, 8, T) + dzn4
            big[prow(t, 1), :] = _dual_softmax_bwd(fp, fn, dp, dm).astype(BF)
            dw = dw + _nt(xnT[:, pl.ds(t * T, T)], big[_rows(t * G + g, 384), :])
        dwq, dwk = dw[:, 0:128].astype(BF), dw[:, 128:256].astype(BF)
        dphi_w = jnp.where(_diag_mask(128), _tn(wqkv[0, g], dwq) + _tn(wqkv[1, g], dwk), 0.0)
        dwphi_ref[_rows(g, 128), :] = (dphi_w[:, 0:32] + dphi_w[:, 32:64]
                                       + dphi_w[:, 64:96] + dphi_w[:, 96:128]).astype(BF)
        wqkv[0, g] = _nt(dwq, bd[g]).astype(BF)
        wqkv[1, g] = _nt(dwk, bd[g]).astype(BF)
        wqkv[2, g] = dw[:, 256:384].astype(BF)
        for j in range(3):
            dqkv_cp(j, g).start()

    lax.fori_loop(0, G, att_bwd, None)

    def dx(t, _):
        r = _rows(t, T)
        d = _nn(wall[...], big[_rows(t, 3 * D), :]).T + acc[r, :]
        n = xn[r, :].astype(F32)
        d = d - jnp.mean(d, axis=-1, keepdims=True) - n * jnp.mean(d * n, axis=-1, keepdims=True)
        gob[r, :] = (gob[r, :].astype(F32) + rstd[r, :] * d).astype(BF)
        dx_cp(t).start()

    lax.fori_loop(0, NT_, dx, None)

    dwo_cp.wait()
    for c in range(NC):
        dw1_cp(I(c)).wait()
        dw2_cp(I(c)).wait()
    for j in range(3):
        for g in range(G):
            dqkv_cp(j, I(g)).wait()
    for t in range(NT_):
        out_cp(I(t)).wait()
        dx_cp(I(t)).wait()


@jax.jit
def pallas_recurrent_scan__linear_kernel_hedgehog__dense_activation_relu__prompt_kernel(
    A_x: jax.Array,
    A_wqkv: jax.Array,
    A_w_phi: jax.Array,
    A_wo: jax.Array,
    B_x: jax.Array,
    B_w1: jax.Array,
    B_w2: jax.Array,
    grad_out: jax.Array,
):
    del B_x
    hbm = pl.BlockSpec(memory_space=pl.ANY)
    vmem = pl.BlockSpec(memory_space=pltpu.VMEM)
    V, sem = pltpu.VMEM, pltpu.SemaphoreType.DMA
    sds = jax.ShapeDtypeStruct
    out, dx, dwqkv, dwphi, dwo, dw1, dw2 = pl.pallas_call(
        _kernel,
        in_specs=[hbm, hbm, vmem, hbm, hbm, hbm, hbm],
        out_specs=[hbm, hbm, hbm, vmem, hbm, hbm, hbm],
        out_shape=[sds((S, D), BF), sds((S, D), BF), sds((D, 3 * D), BF), sds((H * DH, DH), BF),
                   sds((D, D), BF), sds((D, F), BF), sds((F, D), BF)],
        scratch_shapes=[
            V((S, D), BF), V((S, D), BF), V((S, D), BF), V((D, S), BF), V((S, 1), F32),
            V((3, G, D, 128), BF), V((D, 3 * D), BF), V((3 * D, D), BF), V((G, 128, 128), BF),
            V((D, D), BF), V((NC, D, FC), BF), V((NC, FC, D), BF),
            V((NC * S, FC), BF), V((S, D), F32),
            V((NT_, G, 256, T), BF), V((NT_, G, 256, T), BF), V((NT_, G, 128, T), BF),
            V((NT_, D, T), BF), V((S, D), BF), V((NT_, D, T), BF), V((S, FC), BF),
            V((G, 256, 128), BF), V((G, 256, 128), F32), V((NT_, H, 8, T), F32),
            sem((NT_,)), sem((NT_,)), sem((3 * G,)), sem((1,)), sem((NC,)), sem((NC,)),
        ],
        compiler_params=pltpu.CompilerParams(vmem_limit_bytes=127 * 1024 * 1024),
    )(A_x.reshape(S, D), A_wqkv, A_w_phi.reshape(H * DH, DH), A_wo, B_w1, B_w2, grad_out.reshape(S, D))
    return (out.reshape(1, S, D), dx.reshape(1, S, D), dwqkv, dwphi.reshape(H, DH, DH), dwo, dw1, dw2)
```

```python
import jax
import jax.numpy as jnp
from jax import lax
import jax.experimental.pallas as pl
import jax.experimental.pallas.tpu as pltpu

S, D, H, DH, F = 2048, 1024, 32, 32, 3584
T = 512
HS, HD = S // 2, D // 2
R = 256
NR = S // R
FC = 512
NC = F // FC
HF = FC // 2
HG = D // 256
G = D // 128
TM = 512
TB = 256
RC = 32
BF, F32 = jnp.bfloat16, jnp.float32


def _nn(a, b):
    return lax.dot_general(a, b, (((1,), (0,)), ((), ())), preferred_element_type=F32)


def _nt(a, b):
    return lax.dot_general(a, b, (((1,), (1,)), ((), ())), preferred_element_type=F32)


def _tn(a, b):
    return lax.dot_general(a, b, (((0,), (0,)), ((), ())), preferred_element_type=F32)


_B = (0, 2, 6, 5, 3, 4, 1)


def _set7(x11, x12, x21, x22):
    return [v.astype(BF) for v in (x11 + x22, x21 + x22, x11, x22, x11 + x12, x21 - x11, x12 - x22)]


def _set7t(x11, x12, x21, x22):
    return _set7(x11, x21, x12, x22)


def _lazy7(blk):
    f = lambda a, b: blk(a, b).astype(F32)
    return lambda i: (lambda: (f(0, 0) + f(1, 1)).astype(BF), lambda: (f(1, 0) + f(1, 1)).astype(BF),
                      lambda: blk(0, 0), lambda: blk(1, 1), lambda: (f(0, 0) + f(0, 1)).astype(BF),
                      lambda: (f(1, 0) - f(0, 0)).astype(BF), lambda: (f(0, 1) - f(1, 1)).astype(BF))[i]()


_TERMS = {(0, 0): {0: 1, 3: 1, 4: -1, 6: 1}, (0, 1): {2: 1, 4: 1}, (1, 0): {1: 1, 3: 1}, (1, 1): {0: 1, 1: -1, 2: 1, 5: 1}}


def _combine(prod, order):
    part, left = {}, {q: len(t) for q, t in _TERMS.items()}
    for i in order:
        m = prod(i)
        for q, terms in _TERMS.items():
            if i in terms:
                sign, v = part.get(q, (terms[i], None))
                if v is None:
                    part[q] = (sign, m)
                elif sign > 0:
                    part[q] = (1, v + m if terms[i] > 0 else v - m)
                else:
                    part[q] = (1, m - v)
                left[q] -= 1
                if not left[q]:
                    yield q, part[q][1]


def _strassen(dot, a, b, order=(4, 2, 1, 3, 0, 5, 6)):
    return _combine(lambda i: dot(a(i), b(_B[i])), order)


def _strassen_t(dot, u, v, order=(2, 4, 3, 1, 0, 5, 6)):
    return (((b, a), x) for (a, b), x in _combine(lambda i: dot(u(_B[i]), v(i)), order))


class _Weave:
    def __init__(self):
        self.todo = []

    def add(self, steps):
        self.todo.append(steps)

    def fill(self, n=1):
        while n and self.todo:
            if next(self.todo[0], self) is self:
                self.todo.pop(0)
            else:
                n -= 1

    def dot(self, dot, parts, n=1):
        def woven(a, b):
            axis = 0 if dot is _nt else 1
            w, out = b.shape[axis] // parts, []
            for k in range(parts):
                out.append(dot(a, lax.slice_in_dim(b, k * w, (k + 1) * w, axis=axis)))
                self.fill(n)
            return jnp.concatenate(out, axis=1)

        return woven


def _zero(p, k):
    return lax.shift_right_logical(p, 3 + k)


def _ahead(items):
    items = iter(items)
    prev = next(items)
    for item in items:
        yield prev
        prev = item
    yield prev


_Q = ((0, 0), (0, 1), (1, 0), (1, 1))


def _rows(i, n):
    if isinstance(i, int):
        return pl.ds(i * n, n)
    return pl.ds(pl.multiple_of(i * n, n), n)


def _seg(op, p4):
    return op(op(p4, axis=1), axis=1, keepdims=True)


def _dual_softmax(p):
    p4 = p.reshape(4, 4, 8, p.shape[-1])
    ep = jnp.exp(p4 - _seg(jnp.max, p4)[:, None])
    en = jnp.exp(_seg(jnp.min, p4)[:, None] - p4)
    return ep * (1.0 / _seg(jnp.sum, ep))[:, None], en * (1.0 / _seg(jnp.sum, en))[:, None]


def _dual_softmax_bwd(fp, fn, dp, dn):
    tp, tn = fp * dp, fn * dn
    r = (tp - fp * _seg(jnp.sum, tp)[:, None]) - (tn - fn * _seg(jnp.sum, tn)[:, None])
    return r.reshape(128, r.shape[-1])


def _stack(p, n):
    return jnp.stack([p, n], axis=1).reshape(256, p.shape[-1])


def _unstack(v):
    v = v.astype(F32).reshape(4, 2, 4, 8, v.shape[-1])
    return v[:, 0], v[:, 1]


def _outer(v, f):
    return jnp.concatenate([_nt(v[0:64], f[0:128]), _nt(v[64:128], f[128:256])], axis=0)


def _apply(k, f):
    return jnp.concatenate([_nn(k[0:64], f[0:128]), _nn(k[64:128], f[128:256])], axis=0)


def _per_head(k):
    r = lax.broadcasted_iota(jnp.int32, (128, 128), 0)
    c = lax.broadcasted_iota(jnp.int32, (128, 128), 1)
    k = jnp.where((r // DH) % 2 == c // (2 * DH), k, 0.0)
    kt = k.T
    return k.astype(BF), jnp.concatenate([jnp.where(c < 64, kt, 0.0), jnp.where(c < 64, 0.0, kt)], axis=0).astype(BF)


def _fold_lanes(v):
    out = v[..., 0:128]
    for i in range(1, v.shape[-1] // 128):
        out = out + v[..., i * 128:(i + 1) * 128]
    return out


def _lane_total(v):
    return jnp.broadcast_to(jnp.sum(v, axis=-1, keepdims=True), v.shape)


def _tile4(z, t):
    return jnp.concatenate([z] * (t // 128), axis=-1).reshape(4, 4, 8, t)


def _diag_mask(rows):
    r = lax.broadcasted_iota(jnp.int32, (rows, 128), 0)
    c = lax.broadcasted_iota(jnp.int32, (rows, 128), 1)
    return ((r % 128) // DH) == (c // DH)


def _kernel(x_hbm, wqkv_hbm, wphi_hbm, wo_hbm, w1_hbm, w2_hbm, go_hbm,
            out_hbm, dx_hbm, dwqkv_hbm, dwphi_hbm, dwo_hbm, dw1_hbm, dw2_hbm,
            xb, gob, xnT7, wqkv, bd, wo, w1, w2, acc, phik, phiq, vT, oT, kvb, zb, rden, wtq, wtk, wtv, wphi,
            s_x, s_go, s_qkv, s_wo, s_w1, s_w2):
    cp = pltpu.make_async_copy
    x_cp = lambda t: cp(x_hbm.at[_rows(t, R)], xb.at[_rows(t, R)], s_x.at[t])
    out_cp = lambda t: cp(xb.at[_rows(t, R)], out_hbm.at[_rows(t, R)], s_x.at[t])
    go_cp = lambda t: cp(go_hbm.at[_rows(t, R)], gob.at[_rows(t, R)], s_go.at[t])
    dx_cp = lambda t: cp(gob.at[_rows(t, R)], dx_hbm.at[_rows(t, R)], s_go.at[t])
    qkv_cp = lambda j, g: cp(wqkv_hbm.at[:, _rows(j * G + g, 128)], wqkv.at[j, g], s_qkv.at[j * G + g])
    dqkv_cp = lambda j, g: cp(wqkv.at[j, g], dwqkv_hbm.at[:, _rows(j * G + g, 128)], s_qkv.at[j * G + g])
    wo_cp = cp(wo_hbm, wo, s_wo.at[0])
    dwo_cp = cp(wo, dwo_hbm, s_wo.at[0])
    wphi_cp = cp(wphi_hbm, wphi, s_wo.at[1])
    dwphi_cp = cp(wphi, dwphi_hbm, s_wo.at[1])
    w1_cp = lambda c: cp(w1_hbm.at[:, _rows(c, FC)], w1.at[c], s_w1.at[c])
    dw1_cp = lambda c: cp(w1.at[c], dw1_hbm.at[:, _rows(c, FC)], s_w1.at[c])
    w2_cp = lambda c: cp(w2_hbm.at[_rows(c, FC)], w2.at[c], s_w2.at[c])
    dw2_cp = lambda c: cp(w2.at[c], dw2_hbm.at[_rows(c, FC)], s_w2.at[c])
    I = jnp.int32

    wphi_cp.start()
    x_cp(0).start()
    x_cp(NR // 2).start()
    w1_cp(0).start()

    def normed(r):
        xv = xb[r, :].astype(F32)
        xc = xv - jnp.mean(xv, axis=-1, keepdims=True)
        rs = 1.0 / jnp.sqrt(jnp.mean(xc * xc, axis=-1, keepdims=True) + 1e-5)
        return xc * rs, rs

    def ln(xn, p):
        nt = []
        for t in (p, p + NR // 2):
            ns = []
            for k in range(R // RC):
                r = _rows(t * (R // RC) + k, RC)
                ns.append(normed(r)[0])
                xn[r, :] = ns[-1].astype(BF)
            nt.append(jnp.concatenate(ns, axis=0).T)
        for i, v in enumerate(_set7t(nt[0][:HD], nt[1][:HD], nt[0][HD:], nt[1][HD:])):
            xnT7[i, :, _rows(p, R)] = v

    wphi_cp.wait()
    for g in range(G):
        wp = wphi[_rows(g, 128), :].astype(F32)
        bd[g] = jnp.where(_diag_mask(128), jnp.concatenate([wp] * 4, axis=1), 0.0).T.astype(BF)
    x_cp(0).wait()
    x_cp(NR // 2).wait()
    w2_cp(0).start()
    x_cp(1).start()
    x_cp(1 + NR // 2).start()

    def accum(ref, idx, first, v):
        ref[idx] = jnp.where(first, v, ref[idx] + v)

    def folded(j, g):
        return _nt(bd[g], wqkv[j, g]) if j < 2 else wqkv[j, g].T.astype(F32)

    def attention():
        for j in range(3):
            for g in range(G):
                qkv_cp(j, g).wait()

        def att_fwd(p, _):
            gs = (p, p + HG)
            for j, wt in ((1, wtk), (0, wtq), (2, wtv)):
                wa, wb = (folded(j, g) for g in gs)
                for i, v in enumerate(_set7t(wa[:, :HD], wa[:, HD:], wb[:, :HD], wb[:, HD:])):
                    wt[i, _rows(p, 128), :] = v

            def project(wt, k):
                for t in range(HS // T):
                    for (a, b), r in _strassen_t(wv.dot(_nn, 2), lambda i: wt[i + _zero(p, t), _rows(p, 128), :],
                                                 lambda i: xnT7[i + _zero(p, k), :, _rows(t, T)], (4, 2, 1, 3, 0, 5, 6)):
                        yield a, t + b * (HS // T), r

            kv = [jnp.zeros((128, 128), F32)] * 2
            zp = [jnp.zeros((128, 128), F32)] * 2
            zn = [jnp.zeros((128, 128), F32)] * 2
            wv = _Weave()

            def lanes(t, v):
                for n in range(T // 128):
                    yield _rows(t * (T // 128) + n, 128), v[:, 128 * n:128 * n + 128]

            def keys(a, t, k):
                for c, v in lanes(t, k):
                    kp, kn = _dual_softmax(v)
                    zp[a], zn[a] = zp[a] + kp.reshape(128, 128), zn[a] + kn.reshape(128, 128)
                    phik[gs[a], :, c] = _stack(kp, kn).astype(BF)
                    yield

            def queries(a, t, q):
                for c, v in lanes(t, q):
                    pq[a, t].append(_stack(*_dual_softmax(v)).astype(BF))
                    phiq[gs[a], :, c] = pq[a, t][-1]
                    yield

            pq = {(a, t): [] for a in range(2) for t in range(S // T)}
            for k, q, (a, t, v) in zip(project(wtk, 0), project(wtq, 1), project(wtv, 2)):
                wv.add(keys(*k))
                wv.add(queries(*q))
                vT[gs[a], :, _rows(t, T)] = v.astype(BF)
            wv.fill(-1)
            for a, g in enumerate(gs):
                kv[a] = _outer(vT[g], phik[g])
            for a, g in enumerate(gs):
                kv[a], kvb[g] = _per_head(kv[a])
                zp[a], zn[a] = _lane_total(zp[a]), _lane_total(zn[a])
                zb[g, 0:128, :] = zp[a]
                zb[g, 128:256, :] = zn[a]
            for a, t in pq:
                for n, f in enumerate(pq[a, t]):
                    g, c = gs[a], _rows(t * (T // 128) + n, 128)
                    fp, fn = _unstack(f)
                    rd = 1.0 / (_seg(jnp.sum, fp * _tile4(zp[a], 128) + fn * _tile4(zn[a], 128)) + 1e-6)
                    rden[_rows(g, 4), :, c] = jnp.broadcast_to(rd, (4, 8, 128))
                    o = _apply(kv[a], f).reshape(4, 4, 8, 128) * rd[:, None]
                    oT[_rows(g, 128), c] = o.reshape(128, 128).astype(BF)

        lax.fori_loop(0, HG, att_fwd, None)

    def gating(dy7, dwo, wo7):
        wo_cp.wait()
        for i in range(7):
            wo7[i] = _lazy7(lambda a, b: wo[_rows(b, HD), _rows(a, HD)])(i)

        def gate(p, _):
            ts = (p, p + NR // 2)
            for t in ts:
                go_cp(t).wait()
            oq = {(a, b): oT[_rows(a, HD), _rows(ts[b], R)] for a, b in _Q}
            o7 = [_lazy7(lambda a, b: oq[a, b])(i) for i in range(7)]
            wv, ds = _Weave(), []

            def chunks(z):
                for k in range(R // 16):
                    quads = []
                    for a, b in _Q:
                        r, c = _rows((ts[a] + z) * (R // 16) + k, 16), _rows(b, HD)
                        y = acc[r, c]
                        sig = 0.5 * jnp.tanh(0.5 * y) + 0.5
                        quads.append((a, b, r, c, gob[r, c].astype(F32), sig, y * sig))
                    yield k, quads

            def before():
                for k, quads in chunks(0):
                    yield ds.append(_set7(*(gv * gt for *_, gv, sig, gt in quads)))

            def after():
                for k, quads in chunks(_zero(p, 0)):
                    dy = []
                    for a, b, r, c, gv, sig, gt in quads:
                        s = sq[a, b][16 * k:16 * k + 16]
                        xb[r, c] = (xb[r, c].astype(F32) + s * gt).astype(BF)
                        dy.append(gv * (sig + gt * (1.0 - sig)) * s)
                    for i, v in enumerate(_set7t(*dy)):
                        dy7[i, _rows(p * (R // 16) + k, 16), :] = v
                    yield

            def heads(a, b, do):
                for k in range(HG):
                    hs, r, c = _rows(a * HG + k, 4), _rows(a * HG + k, 128), _rows(ts[b] + _zero(p, 1), R)
                    dn = do[128 * k:128 * k + 128].reshape(4, 4, 8, R) * rden[hs, :, c][:, None]
                    dd = -_seg(jnp.sum, dn * oT[r, c].astype(F32).reshape(4, 4, 8, R))
                    oT[r, c] = dn.reshape(128, R).astype(BF)
                    rden[hs, :, c] = jnp.broadcast_to(dd, (4, 8, R))
                    yield

            wv.add(before())
            sq = dict(_strassen_t(_tn, lambda i: o7[i], lambda i: wo7[i]))
            wv.fill(-1)
            ds7 = [jnp.concatenate([d[i] for d in ds], axis=0) for i in range(7)]
            wv.add(after())
            for (a, b), do in _strassen_t(wv.dot(_nt, 2), lambda i: wo7[i + _zero(p, 2)], lambda i: ds7[i]):
                wv.add(heads(a, b, do))
            for (a, b), v in _strassen(wv.dot(_nn, 4), lambda i: o7[i], lambda i: ds7[i]):
                accum(dwo, (_rows(a, HD), _rows(b, HD)), p == 0, v)
            wv.fill(-1)
            for t in ts:
                out_cp(t).start()

        lax.fori_loop(0, NR // 2, gate, None)
        wo[...] = dwo[...].astype(BF)
        dwo_cp.start()

    def ffn(act):
        w1_7 = lambda c: _lazy7(lambda a, b: w1[c, _rows(a, HD), _rows(b, HF)])
        w2_7 = lambda c: _lazy7(lambda a, b: w2[c, _rows(a, HF), _rows(b, HD)])

        def forward(xn):
            def ffn_tile(c, m, n):
                aq = []
                for a in range(2):
                    r = _rows(m + a * (HS // n), n)
                    h = _nn(xn[r, :], w1[c])
                    bits = jnp.where(h < 0, I(-2 ** 31), pltpu.bitcast(h, I) & I(2 ** 31 - 1))
                    v = pltpu.bitcast(bits, F32)
                    act[c, r, :] = v.astype(BF)
                    aq += [v[:, :HF], v[:, HF:]]
                a7 = _set7(*aq)
                for (a, b), y in _strassen(_nn, lambda i: a7[i], w2_7(c)):
                    yield (_rows(m + a * (HS // n), n), _rows(b, HD)), y

            def ffn_first(p, _):
                @pl.when(p + 1 < NR // 2)
                def _():
                    x_cp(p + 1).wait()
                    x_cp(p + 1 + NR // 2).wait()

                @pl.when(p + 2 < NR // 2)
                def _():
                    x_cp(p + 2).start()
                    x_cp(p + 2 + NR // 2).start()

                @pl.when(p == 1)
                def _():
                    w1_cp(1).start()
                    w2_cp(1).start()

                for idx, y in ffn_tile(0, p, R):
                    acc[idx] = y
                ln(xn, jnp.minimum(p + 1, NR // 2 - 1))

            def ffn_fwd(c, _):
                w1_cp(c).wait()
                w2_cp(c).wait()
                for m in range(HS // TM):
                    for idx, y in ffn_tile(c, m, TM):
                        acc[idx] += y

            ln(xn, 0)
            w1_cp(0).wait()
            w2_cp(0).wait()
            lax.fori_loop(0, NR // 2, ffn_first, None)
            for c in range(2, NC):
                w1_cp(c).start()
                w2_cp(c).start()
            for j in range(3):
                for g in range(G):
                    qkv_cp(j, g).start()
            wo_cp.start()
            for t in range(NR):
                go_cp(t).start()
            lax.fori_loop(1, NC, ffn_fwd, None)

        pl.run_scoped(forward, pltpu.VMEM((S, D), BF))
        attention()

        def backward(dy7):
            pl.run_scoped(lambda *r: gating(dy7, *r), pltpu.VMEM((D, D), F32), pltpu.VMEM((7, HD, HD), BF))
            for t in range(NR):
                out_cp(t).wait()
            blk = lambda i, m: (_rows((i // 4) * (HS // TB) + m, TB), _rows(i % 4, HF))
            full = lambda i: (_rows(i // 4, HS), _rows(i % 4, HF))

            def ffn_bwd(c, _):
                def dhidden(m):
                    d = {}
                    for (a, b), da in _strassen_t(_nt, lambda i: dy7[i, _rows(m, TB), :], w2_7(c)):
                        bits = pltpu.bitcast(act[c, _rows(m + a * (HS // TB), TB), _rows(b, HF)].astype(F32), I)
                        d[a, b] = jnp.where(bits < 0, 0.0, jnp.where(bits == 0, 0.5 * da, da))
                    d7 = _set7t(*(d[q] for q in _Q))
                    for i, v in enumerate(d7):
                        xb[blk(i, m)] = v
                    return d7

                def dinput(m, d7):
                    for (a, b), v in _strassen_t(_nt, lambda i: d7[i], w1_7(c)):
                        accum(acc, (_rows(m + a * (HS // TB), TB), _rows(b, HD)), c == 0, v)

                def tile(m, _):
                    for k, d7 in [(k, dhidden(k)) for k in (2 * m, 2 * m + 1)]:
                        dinput(k, d7)

                lax.fori_loop(0, HS // TB // 2, tile, None)

                def wgrad(k, _):
                    a7 = _lazy7(lambda a, b: act[c, _rows(a, HS), _rows(b, HF)])
                    for (a, b), v in _strassen_t(_nn, lambda i: xnT7[i, _rows(k, HD // 2), :], lambda i: xb[full(i)]):
                        w1[c, _rows(2 * a + k, HD // 2), _rows(b, HF)] = v.astype(BF)
                    for (a, b), v in _strassen_t(_tn, a7, lambda i: dy7[i, :, _rows(k, HD // 2)]):
                        w2[c, _rows(a, HF), _rows(2 * b + k, HD // 2)] = v.astype(BF)

                lax.fori_loop(0, 2, wgrad, None)
                dw1_cp(c).start()
                dw2_cp(c).start()

            lax.fori_loop(0, NC, ffn_bwd, None)

        pl.run_scoped(backward, pltpu.VMEM((7, HS, HD), BF))

    pl.run_scoped(ffn, pltpu.VMEM((NC, S, FC), BF))
    for t in range(NR):
        x_cp(t).start()

    def attention_bwd(dpq, dpk, dpv):
        def att_bwd(p, _):
            gs = (p, p + HG)

            tiles = [[(a, gs[a], _rows(t + b * (HS // T), T)) for a, b in _Q] for t in range(HS // T)]

            def put(dp, t, quads):
                for i, v in enumerate(_set7(*quads)):
                    dp[i, _rows(p, 128), _rows(t, T)] = v

            def wgrad(dp, k):
                return _strassen_t(_nt, lambda i: xnT7[i + _zero(p, k)], lambda i: dp[i, _rows(p, 128), :], (2, 4, 6, 3, 0, 1, 5))

            def unfold(j, g, dw):
                e = _tn(wqkv[j, g], dw)
                wqkv[j, g] = _nn(dw, bd[g]).astype(BF)
                return e

            dkv = [jnp.zeros((128, 128), F32)] * 2
            dzp = [jnp.zeros((128, 128), F32)] * 2
            dzn = [jnp.zeros((128, 128), F32)] * 2
            for a, g, c in sorted(sum(tiles, []), key=lambda q: q[0]):
                dkv[a] = dkv[a] + _outer(oT[_rows(g + _zero(p, 0), 128), c], phiq[g + _zero(p, 0), :, c])
            dkvt, dkvb = zip(*map(_per_head, dkv))
            for t, quads in enumerate(tiles):
                put(dpv, t, [_apply(dkvt[a], phik[g + _zero(p, 0), :, c]) for a, g, c in quads])
            dwv = wgrad(dpv, 0)
            for t, quads in enumerate(tiles):
                dq = []
                for n, (a, g, c) in enumerate(quads):
                    dd = rden[_rows(g, 4), :, c][:, None]
                    dp, dm = _unstack(_nn(kvb[g], oT[_rows(g, 128), c]))
                    fp, fn = _unstack(phiq[g, :, c])
                    dzp[a] = dzp[a] + _fold_lanes((fp * dd).reshape(128, T))
                    dzn[a] = dzn[a] + _fold_lanes((fn * dd).reshape(128, T))
                    dq.append(_dual_softmax_bwd(fp, fn, dp + _tile4(zb[g, 0:128, :], T) * dd,
                                                dm + _tile4(zb[g, 128:256, :], T) * dd))
                    if n % 2:
                        (r, b), v = next(dwv)
                        wqkv[2, gs[b], _rows(r, HD), :] = v.astype(BF)
                put(dpq, t, dq)
            dzp, dzn = [[_tile4(_lane_total(v), T) for v in dz] for dz in (dzp, dzn)]
            dwq, dw = wgrad(dpq, 1), {}
            for t, quads in enumerate(tiles):
                dk = []
                for n, (a, g, c) in enumerate(quads):
                    dp, dm = _unstack(_nn(dkvb[a], vT[g, :, c]))
                    dk.append(_dual_softmax_bwd(*_unstack(phik[g, :, c]), dp + dzp[a], dm + dzn[a]))
                    if n % 2:
                        dw.update([next(dwq)])
                put(dpk, t, dk)
            column = lambda b: jnp.concatenate([dw[0, b], dw[1, b]], axis=0).astype(BF)
            es = [unfold(0, g, column(b)) for b, g in enumerate(gs)]
            for (r, b), v in wgrad(dpk, 2):
                dw[r, b] = v
                if r == b:
                    e = jnp.where(_diag_mask(128), es[b] + unfold(1, gs[b], column(b)), 0.0)
                    wphi[_rows(gs[b], 128), :] = (e[:, 0:32] + e[:, 32:64] + e[:, 64:96] + e[:, 96:128]).astype(BF)
            for g in gs:
                for j in range(3):
                    dqkv_cp(j, g).start()

        lax.fori_loop(0, HG, att_bwd, None)

        def dx(p, _):
            ts = (p, p + NR // 2)
            c = _rows(p, R)
            wv, dq = _Weave(), {}
            dot = wv.dot(_tn, 2)

            def rows(a):
                for k in range(R // RC):
                    r, q = _rows(ts[a] * (R // RC) + k, RC), slice(k * RC, (k + 1) * RC)
                    d = jnp.concatenate([dq[a, 0][q], dq[a, 1][q]], axis=1) + acc[r, :]
                    n, rs = normed(r)
                    d = d - jnp.mean(d, axis=-1, keepdims=True) - n * jnp.mean(d * n, axis=-1, keepdims=True)
                    gob[r, :] = (gob[r, :].astype(F32) + rs * d).astype(BF)
                    yield

            for (a, b), v in _strassen_t(
                    lambda i, j: dot(dpq[i, :, c], wtq[j]) + dot(dpk[i, :, c], wtk[j]) + dot(dpv[i, :, c], wtv[j]),
                    lambda i: i, lambda j: j, (1, 3, 6, 4, 0, 2, 5)):
                dq[a, b] = v
                if a == b:
                    wv.add(rows(a))
            wv.fill(-1)
            for t in ts:
                dx_cp(t).start()

        dwphi_cp.start()
        for t in range(NR):
            x_cp(t).wait()
        lax.fori_loop(0, NR // 2, dx, None)

    pl.run_scoped(attention_bwd, *[pltpu.VMEM((7, HD, HS), BF)] * 3)

    dwo_cp.wait()
    dwphi_cp.wait()
    for c in range(NC):
        dw1_cp(c).wait()
        dw2_cp(c).wait()
    for j in range(3):
        for g in range(G):
            dqkv_cp(j, g).wait()
    for t in range(NR):
        dx_cp(t).wait()


@jax.jit
def pallas_recurrent_scan__linear_kernel_hedgehog__dense_activation_relu__prompt_kernel(
    A_x: jax.Array,
    A_wqkv: jax.Array,
    A_w_phi: jax.Array,
    A_wo: jax.Array,
    B_x: jax.Array,
    B_w1: jax.Array,
    B_w2: jax.Array,
    grad_out: jax.Array,
):
    del B_x
    hbm = pl.BlockSpec(memory_space=pl.ANY)
    V, sem = pltpu.VMEM, pltpu.SemaphoreType.DMA
    sds = jax.ShapeDtypeStruct
    out, dx, dwqkv, dwphi, dwo, dw1, dw2 = pl.pallas_call(
        _kernel,
        in_specs=[hbm] * 7,
        out_specs=[hbm] * 7,
        out_shape=[sds((S, D), BF), sds((S, D), BF), sds((D, 3 * D), BF), sds((H * DH, DH), BF),
                   sds((D, D), BF), sds((D, F), BF), sds((F, D), BF)],
        scratch_shapes=[
            V((S, D), BF), V((S, D), BF), V((7, HD, HS), BF),
            V((3, G, D, 128), BF), V((G, 128, 128), BF),
            V((D, D), BF), V((NC, D, FC), BF), V((NC, FC, D), BF), V((S, D), F32),
            V((G, 256, S), BF), V((G, 256, S), BF), V((G, 128, S), BF), V((D, S), BF),
            V((G, 256, 128), BF), V((G, 256, 128), F32), V((H, 8, S), F32),
            V((7, HD, HD), BF), V((7, HD, HD), BF), V((7, HD, HD), BF),
            V((H * DH, DH), BF),
            sem((NR,)), sem((NR,)), sem((3 * G,)), sem((2,)), sem((NC,)), sem((NC,)),
        ],
        compiler_params=pltpu.CompilerParams(vmem_limit_bytes=127 * 1024 * 1024),
    )(A_x.reshape(S, D), A_wqkv, A_w_phi.reshape(H * DH, DH), A_wo, B_w1, B_w2, grad_out.reshape(S, D))
    return (out.reshape(1, S, D), dx.reshape(1, S, D), dwqkv, dwphi.reshape(H, DH, DH), dwo, dw1, dw2)
```

```python
import jax
import jax.numpy as jnp
from jax import lax
import jax.experimental.pallas as pl
import jax.experimental.pallas.tpu as pltpu

S, D, H, DH, F = 2048, 1024, 32, 32, 3584
HS, HD = S // 2, D // 2
T = 512
R = 256
NR = S // R
RC = 32
NH = 2
FC = 512
NC = F // FC
HF = FC // 2
G = D // 128
HG = G // 2
TM, TB = 512, 256
BF, F32 = jnp.bfloat16, jnp.float32


def _nn(a, b):
    return lax.dot_general(a, b, (((1,), (0,)), ((), ())), preferred_element_type=F32)


def _nt(a, b):
    return lax.dot_general(a, b, (((1,), (1,)), ((), ())), preferred_element_type=F32)


def _tn(a, b):
    return lax.dot_general(a, b, (((0,), (0,)), ((), ())), preferred_element_type=F32)


_B = (0, 2, 6, 5, 3, 4, 1)


def _set7(x11, x12, x21, x22):
    return [v.astype(BF) for v in (x11 + x22, x21 + x22, x11, x22, x11 + x12, x21 - x11, x12 - x22)]


def _set7t(x11, x12, x21, x22):
    return _set7(x11, x21, x12, x22)


def _lazy7(blk):
    f = lambda a, b: blk(a, b).astype(F32)
    return lambda i: (lambda: (f(0, 0) + f(1, 1)).astype(BF), lambda: (f(1, 0) + f(1, 1)).astype(BF),
                      lambda: blk(0, 0), lambda: blk(1, 1), lambda: (f(0, 0) + f(0, 1)).astype(BF),
                      lambda: (f(1, 0) - f(0, 0)).astype(BF), lambda: (f(0, 1) - f(1, 1)).astype(BF))[i]()


_TERMS = {(0, 0): {0: 1, 3: 1, 4: -1, 6: 1}, (0, 1): {2: 1, 4: 1}, (1, 0): {1: 1, 3: 1}, (1, 1): {0: 1, 1: -1, 2: 1, 5: 1}}


def _combine(prod, order):
    part, left = {}, {q: len(t) for q, t in _TERMS.items()}
    for i in order:
        m = prod(i)
        for q, terms in _TERMS.items():
            if i in terms:
                sign, v = part.get(q, (terms[i], None))
                if v is None:
                    part[q] = (sign, m)
                elif sign > 0:
                    part[q] = (1, v + m if terms[i] > 0 else v - m)
                else:
                    part[q] = (1, m - v)
                left[q] -= 1
                if not left[q]:
                    yield q, part[q][1]


def _strassen(dot, a, b, order=(4, 2, 1, 3, 0, 5, 6)):
    return _combine(lambda i: dot(a(i), b(_B[i])), order)


def _strassen_t(dot, u, v, order=(2, 4, 3, 1, 0, 5, 6)):
    return (((b, a), x) for (a, b), x in _combine(lambda i: dot(u(_B[i]), v(i)), order))


def _woven(dot, parts, steps):
    def run(a, b):
        w, out = a.shape[0] // parts, []
        for k in range(parts):
            next(steps, None)
            out.append(dot(a[k * w:(k + 1) * w], b))
        return jnp.concatenate(out, axis=0)

    return run


def _zero(p, k):
    return lax.shift_right_logical(p, 3 + k)


_Q = ((0, 0), (0, 1), (1, 0), (1, 1))


def _rows(i, n):
    if isinstance(i, int):
        return pl.ds(i * n, n)
    return pl.ds(pl.multiple_of(i * n, n), n)


def _seg(op, p4):
    return op(op(p4, axis=1), axis=1, keepdims=True)


def _dual_softmax(p):
    p4 = p.reshape(4, 4, 8, p.shape[-1])
    ep = jnp.exp(p4 - _seg(jnp.max, p4)[:, None])
    en = jnp.exp(_seg(jnp.min, p4)[:, None] - p4)
    return ep * (1.0 / _seg(jnp.sum, ep))[:, None], en * (1.0 / _seg(jnp.sum, en))[:, None]


def _dual_softmax_bwd(fp, fn, dp, dn):
    tp, tn = fp * dp, fn * dn
    r = (tp - fp * _seg(jnp.sum, tp)[:, None]) - (tn - fn * _seg(jnp.sum, tn)[:, None])
    return r.reshape(128, r.shape[-1])


def _stack(p, n):
    return jnp.stack([p, n], axis=1).reshape(256, p.shape[-1])


def _unstack(v):
    v = v.astype(F32).reshape(4, 2, 4, 8, v.shape[-1])
    return v[:, 0], v[:, 1]


def _outer(v, f):
    return jnp.concatenate([_nt(v[0:64], f[0:128]), _nt(v[64:128], f[128:256])], axis=0)


def _apply(k, f):
    return jnp.concatenate([_nn(k[0:64], f[0:128]), _nn(k[64:128], f[128:256])], axis=0)


def _per_head(k):
    r = lax.broadcasted_iota(jnp.int32, (128, 128), 0)
    c = lax.broadcasted_iota(jnp.int32, (128, 128), 1)
    k = jnp.where((r // DH) % 2 == c // (2 * DH), k, 0.0)
    kt = k.T
    return k.astype(BF), jnp.concatenate([jnp.where(c < 64, kt, 0.0), jnp.where(c < 64, 0.0, kt)], axis=0).astype(BF)


def _lane_total(v):
    return jnp.broadcast_to(jnp.sum(v, axis=-1, keepdims=True), v.shape)


def _diag_mask(rows):
    r = lax.broadcasted_iota(jnp.int32, (rows, 128), 0)
    c = lax.broadcasted_iota(jnp.int32, (rows, 128), 1)
    return ((r % 128) // DH) == (c // DH)


def _kernel(x_hbm, wqkv_hbm, wphi_hbm, wo_hbm, w1_hbm, w2_hbm, go_hbm,
            out_hbm, dx_hbm, dwqkv_hbm, dwphi_hbm, dwo_hbm, dw1_hbm, dw2_hbm,
            xb, gob, xnT7, wqkv, bd, wo, w1, w2, acc, phik, phiq, vT, oT, kvb, zb, rden, wtq, wtk, wtv, wphi,
            s_x, s_go, s_qkv, s_wo, s_w1, s_w2):
    cp = pltpu.make_async_copy
    x_cp = lambda t: cp(x_hbm.at[_rows(t, R)], xb.at[_rows(t, R)], s_x.at[t])
    out_cp = lambda t: cp(xb.at[_rows(t, R)], out_hbm.at[_rows(t, R)], s_x.at[t])
    go_cp = lambda t: cp(go_hbm.at[_rows(t, R)], gob.at[_rows(t, R)], s_go.at[t])
    dx_cp = lambda t: cp(gob.at[_rows(t, R)], dx_hbm.at[_rows(t, R)], s_go.at[t])
    qkv_cp = lambda j, g: cp(wqkv_hbm.at[:, _rows(j * G + g, 128)], wqkv.at[j, g], s_qkv.at[j * G + g])
    dqkv_cp = lambda j, g: cp(wqkv.at[j, g], dwqkv_hbm.at[:, _rows(j * G + g, 128)], s_qkv.at[j * G + g])
    wo_cp = cp(wo_hbm, wo, s_wo.at[0])
    dwo_cp = cp(wo, dwo_hbm, s_wo.at[0])
    wphi_cp = cp(wphi_hbm, wphi, s_wo.at[1])
    dwphi_cp = cp(wphi, dwphi_hbm, s_wo.at[1])
    w1_cp = lambda c: cp(w1_hbm.at[:, _rows(c, FC)], w1.at[c], s_w1.at[c])
    dw1_cp = lambda c: cp(w1.at[c], dw1_hbm.at[:, _rows(c, FC)], s_w1.at[c])
    w2_cp = lambda c: cp(w2_hbm.at[_rows(c, FC)], w2.at[c], s_w2.at[c])
    dw2_cp = lambda c: cp(w2.at[c], dw2_hbm.at[_rows(c, FC)], s_w2.at[c])
    I = jnp.int32

    wphi_cp.start()
    x_cp(0).start()
    x_cp(NR // 2).start()
    w1_cp(0).start()

    def normed(r):
        xv = xb[r, :].astype(F32)
        xc = xv - jnp.mean(xv, axis=-1, keepdims=True)
        rs = 1.0 / jnp.sqrt(jnp.mean(xc * xc, axis=-1, keepdims=True) + 1e-5)
        return xc * rs, rs

    def ln(xn, p):
        nt = []
        for t in (p, p + NR // 2):
            ns = []
            for k in range(R // RC):
                r = _rows(t * (R // RC) + k, RC)
                ns.append(normed(r)[0])
                xn[r, :] = ns[-1].astype(BF)
            nt.append(jnp.concatenate(ns, axis=0).T)
        for i, v in enumerate(_set7t(nt[0][:HD], nt[1][:HD], nt[0][HD:], nt[1][HD:])):
            xnT7[i, :, _rows(p, R)] = v

    wphi_cp.wait()
    for g in range(G):
        wp = wphi[_rows(g, 128), :].astype(F32)
        bd[g] = jnp.where(_diag_mask(128), jnp.concatenate([wp] * 4, axis=1), 0.0).T.astype(BF)
    x_cp(0).wait()
    x_cp(NR // 2).wait()
    w2_cp(0).start()
    x_cp(1).start()
    x_cp(1 + NR // 2).start()

    def accum(ref, idx, first, v):
        ref[idx] = jnp.where(first, v, ref[idx] + v)

    def folded(j, g):
        return _nt(bd[g], wqkv[j, g]) if j < 2 else wqkv[j, g].T.astype(F32)

    def attention():
        for j in range(3):
            for g in range(G):
                qkv_cp(j, g).wait()

        def att_fwd(p, _):
            gs = (p, p + HG)
            for j, wt in ((1, wtk), (0, wtq), (2, wtv)):
                wa, wb = (folded(j, g) for g in gs)
                for i, v in enumerate(_set7t(wa[:, :HD], wa[:, HD:], wb[:, :HD], wb[:, HD:])):
                    wt[i, _rows(p, 128), :] = v

            def project(wt, k):
                for t in range(HS // T):
                    for (a, b), r in _strassen_t(_nn, lambda i: wt[i + _zero(p, t + 3), _rows(p, 128), :],
                                                 lambda i: xnT7[i + _zero(p, k), :, _rows(t, T)],
                                                 (4, 2, 1, 3, 0, 5, 6)):
                        for n in range(T // 128):
                            yield a, gs[a], _rows((t * T + b * HS) // 128 + n, 128), r[:, 128 * n:128 * n + 128]

            kv = [None] * 2
            zp = [jnp.zeros((4, 4, 8, 128), F32)] * 2
            zn = [jnp.zeros((4, 4, 8, 128), F32)] * 2
            pq = []
            for (a, g, c, k), (_, _, _, q), (_, _, _, v) in zip(project(wtk, 0), project(wtq, 2), project(wtv, 1)):
                kp, kn = _dual_softmax(k)
                zp[a], zn[a] = zp[a] + kp, zn[a] + kn
                phik[g, :, c] = _stack(kp, kn).astype(BF)
                pq.append((a, g, c, _stack(*_dual_softmax(q)).astype(BF)))
                phiq[g, :, c] = pq[-1][3]
                vT[g, :, c] = v.astype(BF)
            for a, g in enumerate(gs):
                kv[a], kvb[g] = _per_head(_outer(vT[g], phik[g]))
                zp[a], zn[a] = _lane_total(zp[a]), _lane_total(zn[a])
                zb[g, 0] = zp[a]
                zb[g, 1] = zn[a]
            for a, g, c, f in sorted(pq, key=lambda v: v[0]):
                fp, fn = _unstack(f)
                rd = 1.0 / (_seg(jnp.sum, fp * zp[a] + fn * zn[a]) + 1e-6)
                rden[_rows(g, 4), :, c] = jnp.broadcast_to(rd, (4, 8, 128))
                o = _apply(kv[a], f).reshape(4, 4, 8, 128) * rd[:, None]
                oT[_rows(g, 128), c] = o.reshape(128, 128).astype(BF)

        lax.fori_loop(0, HG, att_fwd, None)

    def gating(dy7, dwo, wo7):
        wo_cp.wait()
        for i in range(7):
            wo7[i] = _lazy7(lambda a, b: wo[_rows(b, HD), _rows(a, HD)])(i)

        def gate(p, _):
            ts = (p, p + NR // 2)
            for t in ts:
                go_cp(t).wait()
            oq = {(a, b): oT[_rows(a, HD), _rows(ts[b], R)] for a, b in _Q}
            o7 = [_lazy7(lambda a, b: oq[a, b])(i) for i in range(7)]

            def chunks(z):
                for k in range(R // 16):
                    quads = []
                    for a, b in _Q:
                        r, c = _rows((ts[a] + z) * (R // 16) + k, 16), _rows(b, HD)
                        y = acc[r, c]
                        sig = 0.5 * jnp.tanh(0.5 * y) + 0.5
                        quads.append((a, b, r, c, gob[r, c].astype(F32), sig, y * sig))
                    yield k, quads

            sq = dict(_strassen_t(_tn, lambda i: o7[i], lambda i: wo7[i]))
            ds = [_set7(*(gv * gt for *_, gv, sig, gt in quads)) for k, quads in chunks(0)]
            ds7 = [jnp.concatenate([d[i] for d in ds], axis=0) for i in range(7)]
            for k, quads in chunks(_zero(p, 0)):
                dy = []
                for a, b, r, c, gv, sig, gt in quads:
                    s = sq[a, b][16 * k:16 * k + 16]
                    xb[r, c] = (xb[r, c].astype(F32) + s * gt).astype(BF)
                    dy.append(gv * (sig + gt * (1.0 - sig)) * s)
                for i, v in enumerate(_set7t(*dy)):
                    dy7[i, _rows(p * (R // 16) + k, 16), :] = v
            for (a, b), do in _strassen_t(_nt, lambda i: wo7[i + _zero(p, 2)], lambda i: ds7[i]):
                for k in range(HG):
                    hs, r, c = _rows(a * HG + k, 4), _rows(a * HG + k, 128), _rows(ts[b] + _zero(p, 1), R)
                    dn = do[128 * k:128 * k + 128].reshape(4, 4, 8, R) * rden[hs, :, c][:, None]
                    dd = -_seg(jnp.sum, dn * oT[r, c].astype(F32).reshape(4, 4, 8, R))
                    oT[r, c] = dn.reshape(128, R).astype(BF)
                    rden[hs, :, c] = jnp.broadcast_to(dd, (4, 8, R))
            for (a, b), v in _strassen(_nn, lambda i: o7[i], lambda i: ds7[i]):
                accum(dwo, (_rows(a, HD), _rows(b, HD)), p == 0, v)
            for t in ts:
                out_cp(t).start()

        lax.fori_loop(0, NR // 2, gate, None)
        wo[...] = dwo[...].astype(BF)
        dwo_cp.start()

    def ffn(act):
        w1_7 = lambda c: _lazy7(lambda a, b: w1[c, _rows(a, HD), _rows(b, HF)])
        w2_7 = lambda c: _lazy7(lambda a, b: w2[c, _rows(a, HF), _rows(b, HD)])

        def forward(xn):
            def ffn_tile(c, m, n):
                aq = []
                for a in range(2):
                    r = _rows(m + a * (HS // n), n)
                    h = _nn(xn[r, :], w1[c])
                    bits = jnp.where(h < 0, I(-2 ** 31), pltpu.bitcast(h, I) & I(2 ** 31 - 1))
                    v = pltpu.bitcast(bits, F32)
                    act[c, r, :] = v.astype(BF)
                    aq += [v[:, :HF], v[:, HF:]]
                a7 = _set7(*aq)
                for (a, b), y in _strassen(_nn, lambda i: a7[i], w2_7(c)):
                    yield (_rows(m + a * (HS // n), n), _rows(b, HD)), y

            def ffn_first(p, _):
                @pl.when(p + 1 < NR // 2)
                def _():
                    x_cp(p + 1).wait()
                    x_cp(p + 1 + NR // 2).wait()

                @pl.when(p + 2 < NR // 2)
                def _():
                    x_cp(p + 2).start()
                    x_cp(p + 2 + NR // 2).start()

                @pl.when(p == 1)
                def _():
                    w1_cp(1).start()
                    w2_cp(1).start()

                for idx, y in ffn_tile(0, p, R):
                    acc[idx] = y
                ln(xn, jnp.minimum(p + 1, NR // 2 - 1))

            def ffn_fwd(c, _):
                w1_cp(c).wait()
                w2_cp(c).wait()
                for m in range(HS // TM):
                    for idx, y in ffn_tile(c, m, TM):
                        acc[idx] += y

            ln(xn, 0)
            w1_cp(0).wait()
            w2_cp(0).wait()
            lax.fori_loop(0, NR // 2, ffn_first, None)
            for c in range(2, NC):
                w1_cp(c).start()
                w2_cp(c).start()
            for j in range(3):
                for g in range(G):
                    qkv_cp(j, g).start()
            wo_cp.start()
            for t in range(NR):
                go_cp(t).start()
            lax.fori_loop(1, NC, ffn_fwd, None)

        pl.run_scoped(forward, pltpu.VMEM((S, D), BF))
        attention()

        def backward(dy7):
            pl.run_scoped(lambda *r: gating(dy7, *r), pltpu.VMEM((D, D), F32), pltpu.VMEM((7, HD, HD), BF))
            for t in range(NR):
                out_cp(t).wait()
            blk = lambda i, m: (_rows((i // 4) * (HS // TB) + m, TB), _rows(i % 4, HF))
            full = lambda i: (_rows(i // 4, HS), _rows(i % 4, HF))

            def ffn_bwd(c, _):
                def dhidden(m):
                    d = {}
                    for (a, b), da in _strassen_t(_nt, lambda i: dy7[i, _rows(m, TB), :], w2_7(c)):
                        bits = pltpu.bitcast(act[c, _rows(m + a * (HS // TB), TB), _rows(b, HF)].astype(F32), I)
                        d[a, b] = jnp.where(bits < 0, 0.0, jnp.where(bits == 0, 0.5 * da, da))
                    d7 = _set7t(*(d[q] for q in _Q))
                    for i, v in enumerate(d7):
                        xb[blk(i, m)] = v
                    return d7

                def dinput(m, d7):
                    for (a, b), v in _strassen_t(_nt, lambda i: d7[i], w1_7(c)):
                        accum(acc, (_rows(m + a * (HS // TB), TB), _rows(b, HD)), c == 0, v)

                def tile(m, _):
                    for k, d7 in [(k, dhidden(k)) for k in (2 * m, 2 * m + 1)]:
                        dinput(k, d7)

                lax.fori_loop(0, HS // TB // 2, tile, None)

                def wgrad(k, _):
                    a7 = _lazy7(lambda a, b: act[c, _rows(a, HS), _rows(b, HF)])
                    for (a, b), v in _strassen_t(_nn, lambda i: xnT7[i, _rows(k, HD // 2), :], lambda i: xb[full(i)]):
                        w1[c, _rows(2 * a + k, HD // 2), _rows(b, HF)] = v.astype(BF)
                    for (a, b), v in _strassen_t(_tn, a7, lambda i: dy7[i, :, _rows(k, HD // 2)]):
                        w2[c, _rows(a, HF), _rows(2 * b + k, HD // 2)] = v.astype(BF)

                lax.fori_loop(0, 2, wgrad, None)
                dw1_cp(c).start()
                dw2_cp(c).start()

            lax.fori_loop(0, NC, ffn_bwd, None)

        pl.run_scoped(backward, pltpu.VMEM((7, HS, HD), BF))

    pl.run_scoped(ffn, pltpu.VMEM((NC, S, FC), BF))
    for t in range(NR):
        x_cp(t).start()

    def attention_bwd(dpq, dpk, dpv):
        def att_bwd(p, _):
            gs = (p, p + HG)

            tiles = [[(a, gs[a], _rows(t + b * (HS // 128), 128)) for a, b in _Q] for t in range(HS // 128)]

            def put(dp, t, quads):
                for i, v in enumerate(_set7(*quads)):
                    dp[i, _rows(p, 128), _rows(t, 128)] = v

            def wgrad(dp, k, dot=_nt):
                return _strassen_t(dot, lambda i: xnT7[i + _zero(p, k)], lambda i: dp[i, _rows(p, 128), :], (2, 4, 6, 3, 0, 1, 5))

            def unfold(j, g, dw):
                e = _tn(wqkv[j, g], dw)
                wqkv[j, g] = _nn(dw, bd[g]).astype(BF)
                return e

            dzp = [jnp.zeros((4, 4, 8, 128), F32)] * 2
            dzn = [jnp.zeros((4, 4, 8, 128), F32)] * 2
            dkvt, dkvb = zip(*(_per_head(_outer(oT[_rows(g + _zero(p, 0), 128), :], phiq[g + _zero(p, 0)])) for g in gs))
            for t, quads in enumerate(tiles):
                put(dpv, t, [_apply(dkvt[a], phik[g + _zero(p, 0), :, c]) for a, g, c in quads])

            def queries():
                for t, quads in enumerate(tiles):
                    dq = []
                    for a, g, c in quads:
                        dd = rden[_rows(g, 4), :, c][:, None]
                        dp, dm = _unstack(_nn(kvb[g], oT[_rows(g, 128), c]))
                        fp, fn = _unstack(phiq[g, :, c])
                        dzp[a], dzn[a] = dzp[a] + fp * dd, dzn[a] + fn * dd
                        yield dq.append(_dual_softmax_bwd(fp, fn, dp + zb[g, 0] * dd, dm + zb[g, 1] * dd))
                    put(dpq, t, dq)

            def keys():
                zp, zn = [[_lane_total(v) for v in dz] for dz in (dzp, dzn)]
                for t, quads in enumerate(tiles):
                    dk = []
                    for a, g, c in quads:
                        dp, dm = _unstack(_nn(dkvb[a], vT[g, :, c]))
                        yield dk.append(_dual_softmax_bwd(*_unstack(phik[g, :, c]), dp + zp[a], dm + zn[a]))
                    put(dpk, t, dk)

            steps = queries()
            for _ in range(6):
                next(steps)
            for (r, b), v in wgrad(dpv, 0, _woven(_nt, 4, steps)):
                wqkv[2, gs[b], _rows(r, HD), :] = v.astype(BF)
            list(steps)
            steps = keys()
            dw = dict(wgrad(dpq, 1, _woven(_nt, 4, steps)))
            list(steps)
            column = lambda b: jnp.concatenate([dw[0, b], dw[1, b]], axis=0).astype(BF)
            es = [unfold(0, g, column(b)) for b, g in enumerate(gs)]
            for (r, b), v in wgrad(dpk, 2):
                dw[r, b] = v
                if r == b:
                    e = jnp.where(_diag_mask(128), es[b] + unfold(1, gs[b], column(b)), 0.0)
                    wphi[_rows(gs[b], 128), :] = (e[:, 0:32] + e[:, 32:64] + e[:, 64:96] + e[:, 96:128]).astype(BF)
            for g in gs:
                for j in range(3):
                    dqkv_cp(j, g).start()

        lax.fori_loop(0, HG, att_bwd, None)

        def dx(p, _):
            ts = (p, p + NR // 2)
            for h in range(NH):
                c, dq = _rows(NH * p + h, R // NH), {}
                for (a, b), v in _strassen_t(
                        lambda i, j: _tn(dpq[i, :, c], wtq[j]) + _tn(dpk[i, :, c], wtk[j]) + _tn(dpv[i, :, c], wtv[j]),
                        lambda i: i, lambda j: j + _zero(p, h), (1, 3, 6, 4, 0, 2, 5)):
                    dq[a, b] = v
                    if a != b:
                        continue
                    for k in range(R // NH // RC):
                        r, q = _rows((NH * ts[a] + h) * (R // NH // RC) + k, RC), slice(k * RC, (k + 1) * RC)
                        d = jnp.concatenate([dq[a, 0][q], dq[a, 1][q]], axis=1) + acc[r, :]
                        n, rs = normed(r)
                        d = d - jnp.mean(d, axis=-1, keepdims=True) - n * jnp.mean(d * n, axis=-1, keepdims=True)
                        gob[r, :] = (gob[r, :].astype(F32) + rs * d).astype(BF)
            for t in ts:
                dx_cp(t).start()

        dwphi_cp.start()
        for t in range(NR):
            x_cp(t).wait()
        lax.fori_loop(0, NR // 2, dx, None)

    pl.run_scoped(attention_bwd, *[pltpu.VMEM((7, HD, HS), BF)] * 3)

    dwo_cp.wait()
    dwphi_cp.wait()
    for c in range(NC):
        dw1_cp(c).wait()
        dw2_cp(c).wait()
    for j in range(3):
        for g in range(G):
            dqkv_cp(j, g).wait()
    for t in range(NR):
        dx_cp(t).wait()


@jax.jit
def pallas_recurrent_scan__linear_kernel_hedgehog__dense_activation_relu__prompt_kernel(
    A_x: jax.Array,
    A_wqkv: jax.Array,
    A_w_phi: jax.Array,
    A_wo: jax.Array,
    B_x: jax.Array,
    B_w1: jax.Array,
    B_w2: jax.Array,
    grad_out: jax.Array,
):
    del B_x
    hbm = pl.BlockSpec(memory_space=pl.ANY)
    V, sem = pltpu.VMEM, pltpu.SemaphoreType.DMA
    sds = jax.ShapeDtypeStruct
    out, dx, dwqkv, dwphi, dwo, dw1, dw2 = pl.pallas_call(
        _kernel,
        in_specs=[hbm] * 7,
        out_specs=[hbm] * 7,
        out_shape=[sds((S, D), BF), sds((S, D), BF), sds((D, 3 * D), BF), sds((H * DH, DH), BF),
                   sds((D, D), BF), sds((D, F), BF), sds((F, D), BF)],
        scratch_shapes=[
            V((S, D), BF), V((S, D), BF), V((7, HD, HS), BF),
            V((3, G, D, 128), BF), V((G, 128, 128), BF),
            V((D, D), BF), V((NC, D, FC), BF), V((NC, FC, D), BF), V((S, D), F32),
            V((G, 256, S), BF), V((G, 256, S), BF), V((G, 128, S), BF), V((D, S), BF),
            V((G, 256, 128), BF), V((G, 2, 4, 4, 8, 128), F32), V((H, 8, S), F32),
            V((7, HD, HD), BF), V((7, HD, HD), BF), V((7, HD, HD), BF),
            V((H * DH, DH), BF),
            sem((NR,)), sem((NR,)), sem((3 * G,)), sem((2,)), sem((NC,)), sem((NC,)),
        ],
        compiler_params=pltpu.CompilerParams(vmem_limit_bytes=127 * 1024 * 1024),
    )(A_x.reshape(S, D), A_wqkv, A_w_phi.reshape(H * DH, DH), A_wo, B_w1, B_w2, grad_out.reshape(S, D))
    return (out.reshape(1, S, D), dx.reshape(1, S, D), dwqkv, dwphi.reshape(H, DH, DH), dwo, dw1, dw2)
```
